```python
import os as _os
_os.environ.setdefault("JAX_PLATFORMS", "cpu")
import jax
import jax.numpy as jnp

def _softmax(x, axis=-1):
    return jax.nn.softmax(x, axis=axis)
def _gelu(x):
    return jax.nn.gelu(x, approximate=True)
def _silu(x):
    return jax.nn.silu(x)
def _sigmoid(x):
    return jax.nn.sigmoid(x)
def _layernorm(x, axis=-1, eps=1e-5):
    m = jnp.mean(x, axis=axis, keepdims=True)
    v = jnp.var(x, axis=axis, keepdims=True)
    return (x - m) / jnp.sqrt(v + eps)
def _scatter_add(tgt, idx, src, axis=0):
    return tgt.at[idx].add(src)
def _segment_sum(src, seg, n):
    return jax.ops.segment_sum(src, seg, n)
class _Rng:
    def __init__(self, key):
        self._k = key
    def _next(self):
        self._k, sub = jax.random.split(self._k)
        return sub
    def normal(self, shape):
        return jax.random.normal(self._next(), shape, dtype=jnp.bfloat16)
    def randint(self, lo, hi, shape):
        return jax.random.randint(self._next(), shape, lo, hi, dtype=jnp.int32)
    def uniform(self, shape, lo=0.0, hi=1.0):
        return jax.random.uniform(self._next(), shape, jnp.bfloat16, lo, hi)
    def permutation(self, n):
        return jax.random.permutation(self._next(), n)


kernel_name = 'standalone__gqa_softmax__decode'

def setup_inputs():
    _rng = _Rng(jax.random.key(int.from_bytes(__import__("os").urandom(4), "little")))
    _w = (lambda a: (lambda t: t.astype(jnp.bfloat16) if jnp.issubdtype(t.dtype, jnp.floating) else t)(jnp.asarray(a)))
    B, Hq, Hkv, Sq, Sk, D = 8, 32, 32, 1, 4096, 128
    return {
        "q": _w((lambda *s: _rng.normal(s) * 0.4)(B, Hq, Sq, D)),
        "k": _w((lambda *s: _rng.normal(s) * 0.4)(B, Hkv, Sk, D)),
        "v": _w((lambda *s: _rng.normal(s) * 0.05)(B, Hkv, Sk, D)),
    }

def reference(q, k, v):
    B, Hq, Sq, D = q.shape
    Hkv = k.shape[1]
    rep = Hq // Hkv
    k = jnp.repeat(k, rep, axis=1)
    v = jnp.repeat(v, rep, axis=1)
    scale = D ** -0.5
    scores = jnp.einsum("bhqd,bhkd->bhqk", q, k) * scale
    p = _softmax(scores, axis=-1)
    return jnp.einsum("bhqk,bhkd->bhqd", p, v)
```

```python
import functools

import jax
import jax.numpy as jnp
import jax.experimental.pallas as pl
import jax.experimental.pallas.tpu as pltpu

_NBUF = 3
_DESC_ROWS = 128


def _decode_attention_kernel(q_ref, k_hbm, v_hbm, o_ref,
                             kbuf, vbuf, qf, acc, sems,
                             *, n_heads, sk, scale):
    d = q_ref.shape[-1]

    def start(h, slot):
        for r in range(0, sk, _DESC_ROWS):
            for t, (src, dst) in enumerate(((k_hbm, kbuf), (v_hbm, vbuf))):
                pltpu.make_async_copy(
                    src.at[pl.ds(h * sk + r, _DESC_ROWS)],
                    dst.at[slot, pl.ds(r, _DESC_ROWS)],
                    sems.at[slot],
                ).start(priority=t)

    def wait(slot):
        for dst in (kbuf, vbuf):
            pltpu.make_async_copy(dst.at[slot], dst.at[slot], sems.at[slot]).wait()

    for slot in range(_NBUF):
        start(slot, slot)

    qf[...] = q_ref[...].astype(jnp.float32)

    def compute(h, slot):
        q = jnp.broadcast_to(qf[pl.ds(h, 1), :], (8, d)).astype(kbuf.dtype)
        s = jax.lax.dot_general(q, kbuf[slot], (((1,), (1,)), ((), ())),
                                preferred_element_type=jnp.float32) * scale
        m = jnp.max(s, axis=-1, keepdims=True)
        p = jnp.exp(s - m)
        l = jnp.sum(p, axis=-1, keepdims=True)
        o = jnp.dot(p.astype(vbuf.dtype), vbuf[slot],
                    preferred_element_type=jnp.float32)
        acc[pl.ds(h, 1), :] = (o / l)[0:1]

    def body(base, carry):
        for slot in range(_NBUF):
            h = base * _NBUF + slot

            @pl.when(h < n_heads)
            def _():
                wait(slot)
                compute(h, slot)

            @pl.when(h + _NBUF < n_heads)
            def _():
                start(h + _NBUF, slot)
        return carry

    jax.lax.fori_loop(0, pl.cdiv(n_heads, _NBUF), body, 0)
    o_ref[...] = acc[...].astype(o_ref.dtype)


@jax.jit
def pallas_standalone__gqa_softmax__decode_kernel(
    q: jax.Array,
    k: jax.Array,
    v: jax.Array,
):
    B, Hq, Sq, D = q.shape
    Hkv, Sk = k.shape[1], k.shape[2]
    assert Sq == 1 and Hq == Hkv and Sk % _DESC_ROWS == 0
    n_heads = B * Hq
    out = pl.pallas_call(
        functools.partial(_decode_attention_kernel,
                          n_heads=n_heads, sk=Sk, scale=D ** -0.5),
        in_specs=[pl.BlockSpec(memory_space=pltpu.VMEM),
                  pl.BlockSpec(memory_space=pl.ANY),
                  pl.BlockSpec(memory_space=pl.ANY)],
        out_specs=pl.BlockSpec(memory_space=pltpu.VMEM),
        out_shape=jax.ShapeDtypeStruct((n_heads, D), q.dtype),
        scratch_shapes=[pltpu.VMEM((_NBUF, Sk, D), k.dtype),
                        pltpu.VMEM((_NBUF, Sk, D), v.dtype),
                        pltpu.VMEM((n_heads, D), jnp.float32),
                        pltpu.VMEM((n_heads, D), jnp.float32),
                        pltpu.SemaphoreType.DMA((_NBUF,))],
    )(q.reshape(n_heads, D), k.reshape(n_heads * Sk, D), v.reshape(n_heads * Sk, D))
    return out.reshape(B, Hq, Sq, D)
```

```python
import functools

import jax
import jax.numpy as jnp
import jax.experimental.pallas as pl
import jax.experimental.pallas.tpu as pltpu

_NBUF = 3
_DESC_ROWS = 128
_RUN_ROWS = 384


def _decode_attention_kernel(q_ref, k_hbm, v_hbm, o_ref,
                             kbuf, vbuf, qf, acc, ksem, vsem,
                             *, n_heads, sk, scale):
    d = q_ref.shape[-1]
    streams = ((k_hbm, kbuf, ksem), (v_hbm, vbuf, vsem))

    def start(h, slot):
        for r in range(0, sk, _DESC_ROWS):
            for t, (src, dst, sem) in enumerate(streams):
                pltpu.make_async_copy(
                    src.at[pl.ds(h * sk + r, _DESC_ROWS)],
                    dst.at[slot, pl.ds(r, _DESC_ROWS)],
                    sem.at[slot],
                ).start(priority=(r // _RUN_ROWS + t) % 2)

    def wait(slot):
        for _, dst, sem in streams:
            pltpu.make_async_copy(dst.at[slot], dst.at[slot], sem.at[slot]).wait()

    for slot in range(_NBUF):
        start(slot, slot)

    qf[...] = q_ref[...].astype(jnp.float32)

    def compute(h, slot):
        q = jnp.broadcast_to(qf[pl.ds(h, 1), :], (8, d)).astype(kbuf.dtype)
        s = jax.lax.dot_general(q, kbuf[slot], (((1,), (1,)), ((), ())),
                                preferred_element_type=jnp.float32) * scale
        m = jnp.max(s, axis=-1, keepdims=True)
        p = jnp.exp(s - m)
        l = jnp.sum(p, axis=-1, keepdims=True)
        o = jnp.dot(p.astype(vbuf.dtype), vbuf[slot],
                    preferred_element_type=jnp.float32)
        acc[pl.ds(h, 1), :] = (o / l)[0:1]

    def body(base, carry):
        for slot in range(_NBUF):
            h = base * _NBUF + slot

            @pl.when(h < n_heads)
            def _():
                wait(slot)
                compute(h, slot)

            @pl.when(h + _NBUF < n_heads)
            def _():
                start(h + _NBUF, slot)
        return carry

    jax.lax.fori_loop(0, pl.cdiv(n_heads, _NBUF), body, 0)
    o_ref[...] = acc[...].astype(o_ref.dtype)


@jax.jit
def pallas_standalone__gqa_softmax__decode_kernel(
    q: jax.Array,
    k: jax.Array,
    v: jax.Array,
):
    B, Hq, Sq, D = q.shape
    Hkv, Sk = k.shape[1], k.shape[2]
    assert Sq == 1 and Hq == Hkv and Sk % _DESC_ROWS == 0
    n_heads = B * Hq
    out = pl.pallas_call(
        functools.partial(_decode_attention_kernel,
                          n_heads=n_heads, sk=Sk, scale=D ** -0.5),
        in_specs=[pl.BlockSpec(memory_space=pltpu.VMEM),
                  pl.BlockSpec(memory_space=pl.ANY),
                  pl.BlockSpec(memory_space=pl.ANY)],
        out_specs=pl.BlockSpec(memory_space=pltpu.VMEM),
        out_shape=jax.ShapeDtypeStruct((n_heads, D), q.dtype),
        scratch_shapes=[pltpu.VMEM((_NBUF, Sk, D), k.dtype),
                        pltpu.VMEM((_NBUF, Sk, D), v.dtype),
                        pltpu.VMEM((n_heads, D), jnp.float32),
                        pltpu.VMEM((n_heads, D), jnp.float32),
                        pltpu.SemaphoreType.DMA((_NBUF,)),
                        pltpu.SemaphoreType.DMA((_NBUF,))],
    )(q.reshape(n_heads, D), k.reshape(n_heads * Sk, D), v.reshape(n_heads * Sk, D))
    return out.reshape(B, Hq, Sq, D)
```
